```python
import jax
import jax.numpy as jnp

def _softmax(x, axis=-1):
    return jax.nn.softmax(x, axis=axis)

def _gelu(x):
    return jax.nn.gelu(x, approximate=True)

def _silu(x):
    return jax.nn.silu(x)

def _sigmoid(x):
    return jax.nn.sigmoid(x)

def _layernorm(x, axis=-1, eps=1e-05):
    m = jnp.mean(x, axis=axis, keepdims=True)
    v = jnp.var(x, axis=axis, keepdims=True)
    return (x - m) / jnp.sqrt(v + eps)

def _scatter_add(tgt, idx, src, axis=0):
    return tgt.at[idx].add(src)

def _segment_sum(src, seg, n):
    return jax.ops.segment_sum(src, seg, n)

class _Rng:

    def __init__(self, key):
        self._k = key

    def _next(self):
        self._k, sub = jax.random.split(self._k)
        return sub

    def normal(self, shape):
        return jax.random.normal(self._next(), shape, dtype=jnp.bfloat16)

    def randint(self, lo, hi, shape):
        return jax.random.randint(self._next(), shape, lo, hi, dtype=jnp.int32)

    def uniform(self, shape, lo=0.0, hi=1.0):
        return jax.random.uniform(self._next(), shape, jnp.bfloat16, lo, hi)

    def permutation(self, n):
        return jax.random.permutation(self._next(), n)
kernel_name = 'interleave_layers__memory_aug_infini_attn__mixer_s_mlp__prompt'

def setup_inputs():
    _rng = _Rng(jax.random.key(int.from_bytes(__import__("os").urandom(4), "little")))
    _w = lambda a: (lambda t: t.astype(jnp.bfloat16) if jnp.issubdtype(t.dtype, jnp.floating) else t)(jnp.asarray(a))

    def _A_setup():
        B, S, D, H = (1, 2048, 1024, 32)
        N = 4
        L = max(1, S // N)
        sc = D ** (-0.5)
        return {'x': _w((lambda *s: _rng.normal(s) * 0.05)(B, N * L, D)), 'wq': _w((lambda *s: _rng.normal(s) * 0.05)(D, D) * sc), 'wk': _w((lambda *s: _rng.normal(s) * 0.05)(D, D) * sc), 'wv': _w((lambda *s: _rng.normal(s) * 0.05)(D, D) * sc), 'wo': _w((lambda *s: _rng.normal(s) * 0.05)(D, D) * sc), 'beta': _w((lambda *s: _rng.normal(s) * 0.05)(H))}
    _A_in = _A_setup()

    def _B_setup():
        B, S, D, F = (1, 2048, 1024, 3584)
        return {'x': _w((lambda *s: _rng.normal(s) * 0.05)(B, S, D)), 'w1': _w((lambda *s: _rng.normal(s) * 0.05)(D, D) * D ** (-0.5)), 'w2': _w((lambda *s: _rng.normal(s) * 0.05)(D, D) * D ** (-0.5)), 'w3': _w((lambda *s: _rng.normal(s) * 0.05)(D, F) * D ** (-0.5)), 'w4': _w((lambda *s: _rng.normal(s) * 0.05)(F, D) * F ** (-0.5))}
    _B_in = _B_setup()
    return {'A_x': _A_in['x'], 'A_wq': _A_in['wq'], 'A_wk': _A_in['wk'], 'A_wv': _A_in['wv'], 'A_wo': _A_in['wo'], 'A_beta': _A_in['beta'], 'B_x': _B_in['x'], 'B_w1': _B_in['w1'], 'B_w2': _B_in['w2'], 'B_w3': _B_in['w3'], 'B_w4': _B_in['w4']}

def reference(A_x, A_wq, A_wk, A_wv, A_wo, A_beta, B_x, B_w1, B_w2, B_w3, B_w4):

    def _A_ref(x, wq, wk, wv, wo, beta):
        B, S, D = x.shape
        H = 32
        Dh = D // H
        N = 4
        L = S // N
        q = (lambda x, *d: x.transpose(*d))((x @ wq).reshape(B, S, H, Dh), 0, 2, 1, 3).reshape(B, H, N, L, Dh)
        k = (lambda x, *d: x.transpose(*d))((x @ wk).reshape(B, S, H, Dh), 0, 2, 1, 3).reshape(B, H, N, L, Dh)
        v = (lambda x, *d: x.transpose(*d))((x @ wv).reshape(B, S, H, Dh), 0, 2, 1, 3).reshape(B, H, N, L, Dh)
        phi = lambda t: jnp.where(t > 0, t + 1.0, jnp.exp(t))
        scale = Dh ** (-0.5)
        ar = jnp.arange(L)
        mask = (lambda x, dt: x.astype(dt))(ar[:, None] < ar[None, :], x.dtype) * -1000000000.0
        g = _sigmoid(beta).reshape(1, H, 1, 1)
        M = jnp.einsum('bhd,bhe->bhde', q[:, :, 0, 0, :] * 0.0, q[:, :, 0, 0, :] * 0.0)
        z = q[:, :, 0, 0, :] * 0.0
        outs = []
        for s in range(N):
            qs, ks, vs = (q[:, :, s].copy(), k[:, :, s].copy(), v[:, :, s].copy())
            logits = jnp.einsum('bhqd,bhkd->bhqk', qs, ks) * scale + mask
            p = _softmax(logits, axis=-1)
            a_dot = jnp.einsum('bhqk,bhkd->bhqd', p, vs)
            pq = phi(qs)
            num = jnp.einsum('bhld,bhde->bhle', pq, M)
            den = jnp.einsum('bhld,bhd->bhl', pq, z)[..., None] + 1e-06
            a_mem = num / den
            o = g * a_mem + (1.0 - g) * a_dot
            outs.append(o)
            pk = phi(ks)
            M = M + jnp.einsum('bhld,bhle->bhde', pk, vs)
            z = z + jnp.einsum('bhld->bhd', pk)
        o = (lambda x, *d: x.transpose(*d))(jnp.stack(outs, 2).reshape(B, H, S, Dh), 0, 2, 1, 3).reshape(B, S, D)
        return o @ wo

    def _B_ref(x, w1, w2, w3, w4):
        B, S, D = x.shape
        h = _gelu(_layernorm(x, axis=-1) @ w1)
        c = D // 4
        g0 = jnp.pad(h[:, :, 0 * c:1 * c], ((0, 0), (1, 0), (0, 0)))[:, :S, :]
        g1 = jnp.pad(h[:, :, 1 * c:2 * c], ((0, 0), (0, 1), (0, 0)))[:, 1:, :]
        g2 = jnp.pad(h[:, :, 2 * c:3 * c], ((0, 0), (2, 0), (0, 0)))[:, :S, :]
        g3 = jnp.pad(h[:, :, 3 * c:], ((0, 0), (0, 2), (0, 0)))[:, 2:, :]
        hs = jnp.concatenate([g0, g1, g2, g3], axis=-1) @ w2
        x1 = x + hs
        h2 = _gelu(_layernorm(x1, axis=-1) @ w3) @ w4
        return x1 + h2
    x = A_x
    x = x + _A_ref(_layernorm(x, axis=-1), A_wq, A_wk, A_wv, A_wo, A_beta)
    x = x + _B_ref(_layernorm(x, axis=-1), B_w1, B_w2, B_w3, B_w4)
    x = x + _A_ref(_layernorm(x, axis=-1), A_wq, A_wk, A_wv, A_wo, A_beta)
    x = x + _B_ref(_layernorm(x, axis=-1), B_w1, B_w2, B_w3, B_w4)
    return x
```

```python
import numpy as np
import jax
import jax.numpy as jnp
from jax import lax
import jax.experimental.pallas as pl
import jax.experimental.pallas.tpu as pltpu

F32 = jnp.float32
BF16 = jnp.bfloat16
U32 = jnp.uint32

S_, D_, H_, F_ = 2048, 1024, 32, 3584
DH = D_ // H_
NSEG = 4
L_ = S_ // NSEG
NG = D_ // 128
NU = NSEG * NG
EPS = 1e-05
GELU_C0 = float(np.sqrt(2.0 / np.pi))
GELU_C1 = float(0.044715 * np.sqrt(2.0 / np.pi))
QSCALE = float(DH ** -0.5 * np.log2(np.e))
NT = (((1,), (1,)), ((), ()))
XB = 256
RB1 = 256
RB2 = 256
LOGIT_BOUND = 60.0
V_BOUND = float(2.0 ** 40)


def _pack(x):
    return pltpu.bitcast(x.astype(BF16), U32)


def _unpack(x):
    return pltpu.bitcast(x, BF16)


def _ln(x):
    m = jnp.sum(x, axis=1, keepdims=True) * (1.0 / D_)
    d = x - m
    v = jnp.sum(d * d, axis=1, keepdims=True) * (1.0 / D_)
    return d * lax.rsqrt(v + EPS)


def _gelu(x):
    t = jnp.tanh(x * (GELU_C0 + GELU_C1 * (x * x)))
    h = 0.5 * x
    return h + h * t


def _phi(t):
    return jnp.where(t > 0, t + 1.0, jnp.exp(t))


def _dot(a, b):
    return jnp.dot(a, b, preferred_element_type=F32)


def _dot_nt(a, b):
    return lax.dot_general(a, b, NT, preferred_element_type=F32)


def _rows(idx, n):
    return pl.ds(pl.multiple_of(idx * n, n), n)


def _kernel(x_hbm, wq_hbm, wk_hbm, wv_hbm, wo_hbm, beta_ref, w1_hbm, w2_hbm, w3_hbm, w4_hbm,
            out_hbm,
            io_s, wq_s, wk_s, wv_s, wo_s, w1_s, w2_s, w3_s, w4_s,
            x_s, xb_s, xn_s, hp_s, q_s, k_s, pq_s, pk_s, vt_s, o_s, y_s, z2_s, acc_s,
            mt_s, z_s, zk_s, g_s, gl_s, flag_s, x_sem, a_sem, b_sem, out_sem):
    def x_copy(b):
        return pltpu.make_async_copy(x_hbm.at[pl.ds(b * XB, XB), :], io_s.at[pl.ds(b * XB, XB), :], x_sem.at[b])

    def a_copies(g):
        cols = pl.ds(pl.multiple_of(g * 128, 128), 128)
        return [pltpu.make_async_copy(w.at[:, cols], ws.at[g], a_sem.at[j, g])
                for j, (w, ws) in enumerate(((wq_hbm, wq_s), (wk_hbm, wk_s), (wv_hbm, wv_s)))]

    b_copies = [pltpu.make_async_copy(a, b, b_sem.at[i]) for i, (a, b) in
                enumerate(((wo_hbm, wo_s), (w1_hbm, w1_s), (w2_hbm, w2_s), (w3_hbm, w3_s), (w4_hbm, w4_s)))]

    for b in range(S_ // XB):
        x_copy(b).start()
    for g in range(2):
        for c in a_copies(g):
            c.start()

    lane = lax.broadcasted_iota(jnp.int32, (8, 128), 1)
    head_mask = [jnp.where((lane >> 5) == h, jnp.uint32(0xFFFFFFFF), jnp.uint32(0)) for h in range(4)]
    rio = lax.broadcasted_iota(jnp.int32, (128, 128), 0)
    cio = lax.broadcasted_iota(jnp.int32, (128, 128), 1)

    bvec = jax.nn.sigmoid(beta_ref[...].astype(F32))
    hio = lax.broadcasted_iota(jnp.int32, (8, H_), 1)
    for h in range(H_):
        gh = jnp.sum(jnp.where(hio == h, bvec, 0.0), axis=1, keepdims=True)
        g_s[h] = jnp.broadcast_to(gh, (8, 128))

    hp_s[0:8, :] = jnp.zeros((8, D_), U32)
    hp_s[8 + S_ // 2:16 + S_ // 2, :] = jnp.zeros((8, D_), U32)

    def prologue(b, c):
        pltpu.make_async_copy(x_hbm.at[_rows(b, XB), :], io_s.at[_rows(b, XB), :], x_sem.at[b]).wait()
        r = _rows(b, XB)
        x = io_s[r, :].astype(F32)
        x_s[r, :] = x
        xn_s[_rows(b, XB // 2), :] = _pack(_ln(x))
        return c
    lax.fori_loop(0, S_ // XB, prologue, 0)

    for g in range(2, NG):
        for c in a_copies(g):
            c.start()
    for c in b_copies[0:2]:
        c.start()

    def proj_steps(u):
        s, g = u >> 3, u & 7
        tok2 = _rows(s, L_ // 2)
        mx = {}

        def proj(w_ref):
            return _dot(_unpack(xn_s[tok2, :]), w_ref[g])

        def step_q():
            q = proj(wq_s)
            qs = q * QSCALE
            q_s[g] = _pack(qs)
            pq_s[g] = _pack(_phi(q))
            mx['q'] = jnp.max(jnp.abs(qs))

        def step_k():
            k = proj(wk_s)
            k_s[g] = _pack(k)
            pk = _phi(k)
            pk_s[g] = _pack(pk)
            zk_s[g] = jnp.broadcast_to(jnp.sum(pk, axis=0, keepdims=True), (8, 128))
            mx['k'] = jnp.max(jnp.abs(k))

        def step_v():
            v = proj(wv_s)
            vt_s[g] = _pack(v.T)
            bound = (DH * 1.02) * mx['q'] * mx['k']
            ok = jnp.logical_and(bound <= LOGIT_BOUND, jnp.max(jnp.abs(v)) <= V_BOUND)
            flag_s[0] = ok.astype(jnp.int32)
        return [step_q, step_k, step_v]

    def att_unit(u, fillers, safe):
        s, g = u >> 3, u & 7
        fillers = list(fillers)

        def fill():
            if fillers:
                fillers.pop(0)()

        def qk(i):
            nk = 128 * (i + 1)
            kk = _unpack(k_s[g, 0:nk // 2, :])
            qu = q_s[g, i * 64:(i + 1) * 64, :]
            res = []
            for h in range(4):
                qm = _unpack(qu & jnp.concatenate([head_mask[h]] * 8, axis=0))
                st = _dot_nt(kk, qm)
                sd = jnp.where(rio <= cio, st[nk - 128:], -1e30)
                st = jnp.concatenate([st[:nk - 128], sd], axis=0) if i > 0 else sd
                p = jnp.exp2(st)
                res.append((p.astype(BF16), jnp.sum(p, axis=0, keepdims=True)))
            return res

        def pv(i, res):
            nk = 128 * (i + 1)
            outs = []
            for h in range(4):
                p, l = res[h]
                vt = _unpack(vt_s[g, h * 16:(h + 1) * 16, 0:nk])
                outs.append(_dot(vt, p) * (1.0 / l))
            return outs

        def mem_read(i):
            mt = jnp.where((rio >> 5) == (cio >> 5), mt_s[g], 0.0)
            zr = jnp.where(rio[0:16] == (cio[0:16] >> 5), jnp.broadcast_to(z_s[g, 0:1], (16, 128)), 0.0)
            lhs = jnp.concatenate([mt, zr], axis=0).astype(BF16)
            nd = _dot_nt(lhs, _unpack(pq_s[g, i * 64:(i + 1) * 64, :]))
            inv = 1.0 / (nd[128:136] + 1e-06)
            return [nd[h * 32:(h + 1) * 32] * jnp.broadcast_to(inv[h:h + 1], (32, 128)) for h in range(4)]

        def finish(i, adot):
            amem = mem_read(i)
            outs = []
            for h in range(4):
                gh = jnp.concatenate([g_s[g * 4 + h]] * 4, axis=0)
                outs.append(gh * amem[h] + (1.0 - gh) * adot[h])
            ot = jnp.concatenate(outs, axis=0)
            o_s[g, pl.ds(pl.multiple_of(s * (L_ // 2) + i * 64, 64), 64), :] = _pack(ot.T)

        def mem_update():
            mt_s[g] = mt_s[g] + _dot(_unpack(vt_s[g]), _unpack(pk_s[g]))
            z_s[g] = z_s[g] + zk_s[g]

        s3 = qk(3)
        fill()
        s2 = qk(2)
        finish(3, pv(3, s3))
        fill()
        s1 = qk(1)
        finish(2, pv(2, s2))
        fill()
        s0 = qk(0)
        finish(1, pv(1, s1))
        finish(0, pv(0, s0))
        mem_update()

    def att_unit_exact(u):
        s, g = u >> 3, u & 7
        kk = _unpack(k_s[g])
        mt = jnp.where((rio >> 5) == (cio >> 5), mt_s[g], 0.0)
        zr = jnp.where(rio[0:16] == (cio[0:16] >> 5), jnp.broadcast_to(z_s[g, 0:1], (16, 128)), 0.0)
        lhs = jnp.concatenate([mt, zr], axis=0).astype(BF16)
        key = lax.broadcasted_iota(jnp.int32, (L_, 128), 0)
        qry = lax.broadcasted_iota(jnp.int32, (L_, 128), 1)

        def tile(i, c):
            rows = pl.ds(pl.multiple_of(i * 64, 64), 64)
            qu = q_s[g, rows, :]
            nd = _dot_nt(lhs, _unpack(pq_s[g, rows, :]))
            inv = 1.0 / (nd[128:136] + 1e-06)
            outs = []
            for h in range(4):
                qm = _unpack(qu & jnp.concatenate([head_mask[h]] * 8, axis=0))
                st = jnp.where(key <= qry + i * 128, _dot_nt(kk, qm), -1e30)
                p = jnp.exp2(st - jnp.max(st, axis=0, keepdims=True))
                l = jnp.sum(p, axis=0, keepdims=True)
                adot = _dot(_unpack(vt_s[g, h * 16:(h + 1) * 16, :]), p.astype(BF16)) * (1.0 / l)
                amem = nd[h * 32:(h + 1) * 32] * jnp.broadcast_to(inv[h:h + 1], (32, 128))
                gh = jnp.concatenate([g_s[g * 4 + h]] * 4, axis=0)
                outs.append(gh * amem + (1.0 - gh) * adot)
            ot = jnp.concatenate(outs, axis=0)
            o_s[g, pl.ds(pl.multiple_of(s * (L_ // 2) + i * 64, 64), 64), :] = _pack(ot.T)
            return c
        lax.fori_loop(0, 4, tile, 0)
        mt_s[g] = mt_s[g] + _dot(_unpack(vt_s[g]), _unpack(pk_s[g]))
        z_s[g] = z_s[g] + zk_s[g]

    def att_body(t, layer):
        u = t - 1
        nxt = jnp.minimum(t, NU - 1)
        cur = jnp.maximum(u, 0)

        @pl.when(jnp.logical_and(layer == 0, t < NG))
        def _():
            for c in a_copies(t):
                c.wait()

        @pl.when(jnp.logical_and(layer == 0, t == 4))
        def _():
            for c in b_copies[2:]:
                c.start()

        safe = jnp.logical_and(t > 0, flag_s[0] == 1)

        @pl.when(jnp.logical_and(safe, t < NU))
        def _():
            att_unit(cur, proj_steps(nxt), True)

        @pl.when(jnp.logical_and(safe, t == NU))
        def _():
            att_unit(cur, [], True)

        @pl.when(jnp.logical_and(jnp.logical_not(safe), t > 0))
        def _():
            att_unit_exact(cur)

        @pl.when(jnp.logical_and(jnp.logical_not(safe), t < NU))
        def _():
            for st in proj_steps(nxt):
                st()
        return layer

    def out_body(b, c):
        hb = RB1 // 2
        for hf in range(2):
            r = pl.ds(pl.multiple_of(b * RB1 + hf * hb, hb), hb)
            r2 = pl.ds(pl.multiple_of(b * (RB1 // 2) + hf * (hb // 2), hb // 2), hb // 2)
            o = jnp.concatenate([o_s[g, r2, :] for g in range(NG)], axis=1)
            xnew = x_s[r, :] + _dot(_unpack(o), wo_s[...])
            x_s[r, :] = xnew
            xb = _ln(xnew)
            xb_s[r, :] = xb
            y_s[hf * (hb // 2):(hf + 1) * (hb // 2), :] = _pack(_ln(xb))
        for hf in range(2):
            h = _gelu(_dot(_unpack(y_s[hf * (hb // 2):(hf + 1) * (hb // 2), :]), w1_s[...]))
            hp_s[pl.ds(pl.multiple_of(8 + b * (RB1 // 2) + hf * (hb // 2), 8), hb // 2), :] = _pack(h)
        return c

    def mix_body(b, layer):
        n2 = RB2 // 2
        base = pl.multiple_of(b * n2, 8)

        def shifted(c):
            w = hp_s[pl.ds(base, n2 + 16), c * 256:(c + 1) * 256]
            cur = w[8:8 + n2]
            if c == 0:
                return (w[7:7 + n2] >> 16) | (cur << 16)
            if c == 1:
                return (cur >> 16) | (w[9:9 + n2] << 16)
            if c == 2:
                return w[7:7 + n2]
            return w[9:9 + n2]

        for c in range(4):
            y_s[0:n2, c * 256:(c + 1) * 256] = shifted(c)
        hb = RB2 // 2
        h2r = hb // 2
        for hf in range(2):
            r = pl.ds(pl.multiple_of(b * RB2 + hf * hb, hb), hb)
            x1 = xb_s[r, :] + _dot(_unpack(y_s[hf * h2r:(hf + 1) * h2r, :]), w2_s[...])
            acc_s[hf * hb:(hf + 1) * hb, :] = x1
            z2_s[hf * h2r:(hf + 1) * h2r, :] = _pack(_ln(x1))
        for hf in range(2):
            r = pl.ds(pl.multiple_of(b * RB2 + hf * hb, hb), hb)
            z = _unpack(z2_s[hf * h2r:(hf + 1) * h2r, :])
            for ch in range(F_ // 512):
                gl_s[:, ch * 512:(ch + 1) * 512] = _pack(_gelu(_dot(z, w3_s[:, ch * 512:(ch + 1) * 512])))
            h2 = _dot(_unpack(gl_s[...]), w4_s[...])
            xnew = x_s[r, :] + (acc_s[hf * hb:(hf + 1) * hb, :] + h2)
            x_s[r, :] = xnew
            io_s[r, :] = xnew.astype(BF16)
            xn_s[pl.ds(pl.multiple_of(b * n2 + hf * h2r, h2r), h2r), :] = _pack(_ln(xnew))

        @pl.when(layer == 1)
        def _():
            pltpu.make_async_copy(io_s.at[_rows(b, RB2), :], out_hbm.at[_rows(b, RB2), :], out_sem.at[b]).start()
        return layer

    def layer_body(layer, carry):
        mt_s[...] = jnp.zeros(mt_s.shape, F32)
        z_s[...] = jnp.zeros(z_s.shape, F32)
        flag_s[0] = 0
        with jax.named_scope('att'):
            lax.fori_loop(0, NU + 1, att_body, layer)

        @pl.when(layer == 0)
        def _():
            for c in b_copies:
                c.wait()
        with jax.named_scope('out'):
            lax.fori_loop(0, S_ // RB1, out_body, 0)
        with jax.named_scope('mix'):
            lax.fori_loop(0, S_ // RB2, mix_body, layer)
        return carry

    lax.fori_loop(0, 2, layer_body, 0)

    for b in range(S_ // RB2):
        pltpu.make_async_copy(io_s.at[pl.ds(b * RB2, RB2), :], out_hbm.at[pl.ds(b * RB2, RB2), :],
                              out_sem.at[b]).wait()


@jax.jit
def pallas_interleave_layers__memory_aug_infini_attn__mixer_s_mlp__prompt_kernel(
    A_x: jax.Array,
    A_wq: jax.Array,
    A_wk: jax.Array,
    A_wv: jax.Array,
    A_wo: jax.Array,
    A_beta: jax.Array,
    B_x: jax.Array,
    B_w1: jax.Array,
    B_w2: jax.Array,
    B_w3: jax.Array,
    B_w4: jax.Array,
):
    del B_x
    B, S, D = A_x.shape
    assert (B, S, D) == (1, S_, D_) and A_beta.shape == (H_,) and B_w3.shape == (D_, F_)
    hbm = pl.BlockSpec(memory_space=pl.ANY)
    vmem = pl.BlockSpec(memory_space=pltpu.VMEM)
    scratch = [
        pltpu.VMEM((S_, D_), BF16),
        pltpu.VMEM((NG, D_, 128), BF16),
        pltpu.VMEM((NG, D_, 128), BF16),
        pltpu.VMEM((NG, D_, 128), BF16),
        pltpu.VMEM((D_, D_), BF16),
        pltpu.VMEM((D_, D_), BF16),
        pltpu.VMEM((D_, D_), BF16),
        pltpu.VMEM((D_, F_), BF16),
        pltpu.VMEM((F_, D_), BF16),
        pltpu.VMEM((S_, D_), F32),
        pltpu.VMEM((S_, D_), F32),
        pltpu.VMEM((S_ // 2, D_), U32),
        pltpu.VMEM((S_ // 2 + 16, D_), U32),
        pltpu.VMEM((NG, L_ // 2, 128), U32),
        pltpu.VMEM((NG, L_ // 2, 128), U32),
        pltpu.VMEM((NG, L_ // 2, 128), U32),
        pltpu.VMEM((NG, L_ // 2, 128), U32),
        pltpu.VMEM((NG, 64, L_), U32),
        pltpu.VMEM((NG, S_ // 2, 128), U32),
        pltpu.VMEM((max(RB1, RB2) // 2, D_), U32),
        pltpu.VMEM((RB2 // 2, D_), U32),
        pltpu.VMEM((RB2, D_), F32),
        pltpu.VMEM((NG, 128, 128), F32),
        pltpu.VMEM((NG, 8, 128), F32),
        pltpu.VMEM((NG, 8, 128), F32),
        pltpu.VMEM((H_, 8, 128), F32),
        pltpu.VMEM((RB2 // 4, F_), U32),
        pltpu.SMEM((1,), jnp.int32),
        pltpu.SemaphoreType.DMA((S_ // XB,)),
        pltpu.SemaphoreType.DMA((3, NG)),
        pltpu.SemaphoreType.DMA((5,)),
        pltpu.SemaphoreType.DMA((S_ // RB2,)),
    ]
    out = pl.pallas_call(
        _kernel,
        in_specs=[hbm, hbm, hbm, hbm, hbm, vmem, hbm, hbm, hbm, hbm],
        out_specs=hbm,
        out_shape=jax.ShapeDtypeStruct((S_, D_), BF16),
        scratch_shapes=scratch,
        compiler_params=pltpu.CompilerParams(vmem_limit_bytes=100 * 1024 * 1024),
        name="infini_mixer",
    )(A_x.reshape(S_, D_), A_wq, A_wk, A_wv, A_wo, A_beta.reshape(1, H_), B_w1, B_w2, B_w3, B_w4)
    return out.reshape(1, S_, D_)
```

```python
import numpy as np
import jax
import jax.numpy as jnp
from jax import lax
import jax.experimental.pallas as pl
import jax.experimental.pallas.tpu as pltpu

F32 = jnp.float32
BF16 = jnp.bfloat16
U32 = jnp.uint32

S_, D_, H_, F_ = 2048, 1024, 32, 3584
DH = D_ // H_
NSEG = 4
L_ = S_ // NSEG
NG = D_ // 128
NU = NSEG * NG
EPS = 1e-05
GELU_C0 = float(np.sqrt(2.0 / np.pi))
GELU_C1 = float(0.044715 * np.sqrt(2.0 / np.pi))
QSCALE = float(DH ** -0.5 * np.log2(np.e))
NT = (((1,), (1,)), ((), ()))
ORDER = 1
ORD0='kqv'
ORD1='vqk'
XB = 256
RB1 = 256
RB2 = 256
LOGIT_BOUND = 60.0
V_BOUND = float(2.0 ** 40)


def _pack(x):
    return pltpu.bitcast(x.astype(BF16), U32)


def _unpack(x):
    return pltpu.bitcast(x, BF16)


def _ln(x):
    m = jnp.sum(x, axis=1, keepdims=True) * (1.0 / D_)
    d = x - m
    v = jnp.sum(d * d, axis=1, keepdims=True) * (1.0 / D_)
    return d * lax.rsqrt(v + EPS)


def _gelu(x):
    t = jnp.tanh(x * (GELU_C0 + GELU_C1 * (x * x)))
    h = 0.5 * x
    return h + h * t


def _phi(t):
    return jnp.where(t > 0, t + 1.0, jnp.exp(t))


def _dot(a, b):
    return jnp.dot(a, b, preferred_element_type=F32)


def _dot_nt(a, b):
    return lax.dot_general(a, b, NT, preferred_element_type=F32)


def _rows(idx, n):
    return pl.ds(pl.multiple_of(idx * n, n), n)


def _kernel(x_hbm, wq_hbm, wk_hbm, wv_hbm, wo_hbm, beta_ref, w1_hbm, w2_hbm, w3_hbm, w4_hbm,
            out_hbm,
            io_s, wq_s, wk_s, wv_s, wo_s, w1_s, w2_s, w3_s, w4_s,
            x_s, xb_s, xn_s, hp_s, qp0_s, qp1_s, qp2_s, kp0_s, kp1_s, kp2_s, vt0_s, vt1_s, vt2_s, o_s, y_s, z2_s, acc_s,
            mt_s, z_s, zk_s, mx_s, g_s, gl_s, flag_s, x_sem, a_sem, b_sem, out_sem):
    def x_copy(b):
        return pltpu.make_async_copy(x_hbm.at[pl.ds(b * XB, XB), :], io_s.at[pl.ds(b * XB, XB), :], x_sem.at[b])

    def a_copies(g):
        cols = pl.ds(pl.multiple_of(g * 128, 128), 128)
        return [pltpu.make_async_copy(w.at[:, cols], ws.at[g], a_sem.at[j, g])
                for j, (w, ws) in enumerate(((wq_hbm, wq_s), (wk_hbm, wk_s), (wv_hbm, wv_s)))]

    b_copies = [pltpu.make_async_copy(a, b, b_sem.at[i]) for i, (a, b) in
                enumerate(((wo_hbm, wo_s), (w1_hbm, w1_s), (w2_hbm, w2_s), (w3_hbm, w3_s), (w4_hbm, w4_s)))]

    for b in range(S_ // XB):
        x_copy(b).start()
    for g in range(2):
        for c in a_copies(g):
            c.start()

    lane = lax.broadcasted_iota(jnp.int32, (8, 128), 1)
    head_mask = [jnp.where((lane >> 5) == h, jnp.uint32(0xFFFFFFFF), jnp.uint32(0)) for h in range(4)]
    rio = lax.broadcasted_iota(jnp.int32, (128, 128), 0)
    cio = lax.broadcasted_iota(jnp.int32, (128, 128), 1)

    bvec = jax.nn.sigmoid(beta_ref[...].astype(F32))
    hio = lax.broadcasted_iota(jnp.int32, (8, H_), 1)
    for h in range(H_):
        gh = jnp.sum(jnp.where(hio == h, bvec, 0.0), axis=1, keepdims=True)
        g_s[h] = jnp.broadcast_to(gh, (8, 128))

    hp_s[0:8, :] = jnp.zeros((8, D_), U32)
    hp_s[8 + S_ // 2:16 + S_ // 2, :] = jnp.zeros((8, D_), U32)

    def prologue(b, c):
        pltpu.make_async_copy(x_hbm.at[_rows(b, XB), :], io_s.at[_rows(b, XB), :], x_sem.at[b]).wait()
        r = _rows(b, XB)
        x = io_s[r, :].astype(F32)
        x_s[r, :] = x
        xn_s[_rows(b, XB // 2), :] = _pack(_ln(x))
        return c
    lax.fori_loop(0, S_ // XB, prologue, 0)

    for g in range(2, NG):
        for c in a_copies(g):
            c.start()
    for c in b_copies[0:2]:
        c.start()

    qp_b, kp_b, vt_b = (qp0_s, qp1_s, qp2_s), (kp0_s, kp1_s, kp2_s), (vt0_s, vt1_s, vt2_s)

    def proj_steps(u, par, order):
        s, g = u >> 3, u & 7
        tok2 = _rows(s, L_ // 2)

        def proj(w_ref):
            return _dot(_unpack(xn_s[tok2, :]), w_ref[g])

        def absmax(a):
            return jnp.max(jnp.abs(a).reshape(L_ // 8, 8, 128), axis=0)

        def step_q():
            q = proj(wq_s)
            qs = q * QSCALE
            qp_b[par][...] = _pack(jnp.concatenate([qs, _phi(q)], axis=1))
            mx_s[par, 0] = absmax(qs)

        def step_k():
            k = proj(wk_s)
            pk = _phi(k)
            kp_b[par][...] = _pack(jnp.concatenate([k, pk], axis=1))
            zk_s[par] = jnp.broadcast_to(jnp.sum(pk, axis=0, keepdims=True), (8, 128))
            mx_s[par, 1] = absmax(k)

        def step_v():
            v = proj(wv_s)
            vt_b[par][...] = pltpu.bitcast(v.astype(BF16).T, U32)
            mx_s[par, 2] = absmax(v)
        return [dict(q=step_q, k=step_k, v=step_v)[c] for c in order]

    def unit_is_safe(par):
        bound = (DH * 1.02) * jnp.max(mx_s[par, 0]) * jnp.max(mx_s[par, 1])
        return jnp.logical_and(bound <= LOGIT_BOUND, jnp.max(mx_s[par, 2]) <= V_BOUND)

    def mem_lhs(s, g):
        mt = jnp.where((rio >> 5) == (cio >> 5), mt_s[s & 1, g], 0.0)
        zr = jnp.where(rio[0:16] == (cio[0:16] >> 5), jnp.broadcast_to(z_s[s & 1, g, 0:1], (16, 128)), 0.0)
        return jnp.concatenate([mt, zr], axis=0).astype(BF16)

    def mem_update(s, g, par):
        mt_s[1 - (s & 1), g] = mt_s[s & 1, g] + _dot(_unpack(vt_b[par][...]), _unpack(kp_b[par][:, 128:256]))
        z_s[1 - (s & 1), g] = z_s[s & 1, g] + zk_s[par]

    def att_unit(u, par, fillers):
        s, g = u >> 3, u & 7
        fillers = list(fillers)
        safe = unit_is_safe(par)

        def fill():
            if fillers:
                fillers.pop(0)()

        def qk(i):
            nk = 128 * (i + 1)
            kk = _unpack(kp_b[par][0:nk // 2, 0:128])
            qu = qp_b[par][i * 64:(i + 1) * 64, 0:128]
            res = []
            for h in range(4):
                qm = _unpack(qu & jnp.concatenate([head_mask[h]] * 8, axis=0))
                st = _dot_nt(kk, qm)
                sd = jnp.where(rio <= cio, st[nk - 128:], -1e30)
                st = jnp.concatenate([st[:nk - 128], sd], axis=0) if i > 0 else sd
                p = jnp.exp2(st)
                res.append((p.astype(BF16), jnp.sum(p, axis=0, keepdims=True)))
            return res

        def pv(i, res):
            nk = 128 * (i + 1)
            outs = []
            for h in range(4):
                p, l = res[h]
                vt = _unpack(vt_b[par][h * 16:(h + 1) * 16, 0:nk])
                outs.append(_dot(vt, p) * (1.0 / l))
            return outs

        def finish(i, adot):
            nd = _dot_nt(mem_lhs(s, g), _unpack(qp_b[par][i * 64:(i + 1) * 64, 128:256]))
            inv = 1.0 / (nd[128:136] + 1e-06)
            outs = []
            for h in range(4):
                amem = nd[h * 32:(h + 1) * 32] * jnp.broadcast_to(inv[h:h + 1], (32, 128))
                gh = jnp.concatenate([g_s[g * 4 + h]] * 4, axis=0)
                outs.append(gh * amem + (1.0 - gh) * adot[h])
            ot = jnp.concatenate(outs, axis=0)
            o_s[g, pl.ds(pl.multiple_of(s * (L_ // 2) + i * 64, 64), 64), :] = pltpu.bitcast(
                ot.astype(BF16).T, U32)

        if ORDER == 0:
            fill()
            s3 = qk(3)
            s2 = qk(2)
            finish(3, pv(3, s3))
            fill()
            s1 = qk(1)
            finish(2, pv(2, s2))
            s0 = qk(0)
            finish(1, pv(1, s1))
            finish(0, pv(0, s0))
            fill()
        elif ORDER == 1:
            fill()
            s3 = qk(3)
            s0 = qk(0)
            finish(3, pv(3, s3))
            finish(0, pv(0, s0))
            fill()
            s2 = qk(2)
            s1 = qk(1)
            finish(2, pv(2, s2))
            finish(1, pv(1, s1))
            fill()
        elif ORDER == 2:
            fill()
            s3 = qk(3)
            fill()
            s2 = qk(2)
            finish(3, pv(3, s3))
            s1 = qk(1)
            finish(2, pv(2, s2))
            s0 = qk(0)
            finish(1, pv(1, s1))
            finish(0, pv(0, s0))
            fill()
        mem_update(s, g, par)
        flag_s[par] = safe.astype(jnp.int32)

    def att_unit_exact(u, par):
        s, g = u >> 3, u & 7
        kk = _unpack(kp_b[par][:, 0:128])
        lhs = mem_lhs(s, g)
        key = lax.broadcasted_iota(jnp.int32, (L_, 128), 0)
        qry = lax.broadcasted_iota(jnp.int32, (L_, 128), 1)

        def tile(i, c):
            rows = pl.ds(pl.multiple_of(i * 64, 64), 64)
            qu = qp_b[par][rows, 0:128]
            nd = _dot_nt(lhs, _unpack(qp_b[par][rows, 128:256]))
            inv = 1.0 / (nd[128:136] + 1e-06)
            outs = []
            for h in range(4):
                qm = _unpack(qu & jnp.concatenate([head_mask[h]] * 8, axis=0))
                st = jnp.where(key <= qry + i * 128, _dot_nt(kk, qm), -1e30)
                p = jnp.exp2(st - jnp.max(st, axis=0, keepdims=True))
                l = jnp.sum(p, axis=0, keepdims=True)
                adot = _dot(_unpack(vt_b[par][h * 16:(h + 1) * 16, :]), p.astype(BF16)) * (1.0 / l)
                amem = nd[h * 32:(h + 1) * 32] * jnp.broadcast_to(inv[h:h + 1], (32, 128))
                gh = jnp.concatenate([g_s[g * 4 + h]] * 4, axis=0)
                outs.append(gh * amem + (1.0 - gh) * adot)
            ot = jnp.concatenate(outs, axis=0)
            o_s[g, pl.ds(pl.multiple_of(s * (L_ // 2) + i * 64, 64), 64), :] = pltpu.bitcast(
                ot.astype(BF16).T, U32)
            return c
        lax.fori_loop(0, 4, tile, 0)

    def att_body(t, layer):
        NT_ = NU // 2
        ua = jnp.maximum(2 * t - 1, 1)
        ub = jnp.minimum(2 * t, NU - 2)

        @pl.when(jnp.logical_and(layer == 0, t < NG // 2))
        def _():
            for c in a_copies(2 * t) + a_copies(2 * t + 1):
                c.wait()

        @pl.when(jnp.logical_and(layer == 0, t == 2))
        def _():
            for c in b_copies[2:]:
                c.start()

        @pl.when(t == 0)
        def _():
            for st in proj_steps(ub, 0, 'qkv'):
                st()
            flag_s[1] = 1
            att_unit(ub, 0, proj_steps(ub + 1, 1, ORD1))

        @pl.when(jnp.logical_and(t > 0, t < NT_))
        def _():
            att_unit(ua, 1, proj_steps(ub, 0, ORD0))
            att_unit(ub, 0, proj_steps(ub + 1, 1, ORD1))

        @pl.when(t == NT_)
        def _():
            att_unit(ua, 1, [])
            flag_s[0] = 1

        def redo(j, c):
            @pl.when(flag_s[j] == 0)
            def _():
                u = jnp.where(j == 0, ub, ua)
                for st in proj_steps(u, 2, 'qkv'):
                    st()
                att_unit_exact(u, 2)
            return c
        lax.fori_loop(0, 2, redo, 0)
        return layer

    def out_body(b, c):
        hb = RB1 // 2
        for hf in range(2):
            r = pl.ds(pl.multiple_of(b * RB1 + hf * hb, hb), hb)
            r2 = pl.ds(pl.multiple_of(b * (RB1 // 2) + hf * (hb // 2), hb // 2), hb // 2)
            o = jnp.concatenate([o_s[g, r2, :] for g in range(NG)], axis=1)
            xnew = x_s[r, :] + _dot(_unpack(o), wo_s[...])
            x_s[r, :] = xnew
            xb = _ln(xnew)
            xb_s[r, :] = xb
            y_s[hf * (hb // 2):(hf + 1) * (hb // 2), :] = _pack(_ln(xb))
        for hf in range(2):
            h = _gelu(_dot(_unpack(y_s[hf * (hb // 2):(hf + 1) * (hb // 2), :]), w1_s[...]))
            hp_s[pl.ds(pl.multiple_of(8 + b * (RB1 // 2) + hf * (hb // 2), 8), hb // 2), :] = _pack(h)
        return c

    def mix_body(b, layer):
        n2 = RB2 // 2
        base = pl.multiple_of(b * n2, 8)

        def shifted(c):
            w = hp_s[pl.ds(base, n2 + 16), c * 256:(c + 1) * 256]
            cur = w[8:8 + n2]
            if c == 0:
                return (w[7:7 + n2] >> 16) | (cur << 16)
            if c == 1:
                return (cur >> 16) | (w[9:9 + n2] << 16)
            if c == 2:
                return w[7:7 + n2]
            return w[9:9 + n2]

        for c in range(4):
            y_s[0:n2, c * 256:(c + 1) * 256] = shifted(c)
        hb = RB2 // 2
        h2r = hb // 2
        for hf in range(2):
            r = pl.ds(pl.multiple_of(b * RB2 + hf * hb, hb), hb)
            x1 = xb_s[r, :] + _dot(_unpack(y_s[hf * h2r:(hf + 1) * h2r, :]), w2_s[...])
            acc_s[hf * hb:(hf + 1) * hb, :] = x1
            z2_s[hf * h2r:(hf + 1) * h2r, :] = _pack(_ln(x1))
        for hf in range(2):
            r = pl.ds(pl.multiple_of(b * RB2 + hf * hb, hb), hb)
            z = _unpack(z2_s[hf * h2r:(hf + 1) * h2r, :])
            for ch in range(F_ // 512):
                gl_s[:, ch * 512:(ch + 1) * 512] = _pack(_gelu(_dot(z, w3_s[:, ch * 512:(ch + 1) * 512])))
            h2 = _dot(_unpack(gl_s[...]), w4_s[...])
            xnew = x_s[r, :] + (acc_s[hf * hb:(hf + 1) * hb, :] + h2)
            x_s[r, :] = xnew
            io_s[r, :] = xnew.astype(BF16)
            xn_s[pl.ds(pl.multiple_of(b * n2 + hf * h2r, h2r), h2r), :] = _pack(_ln(xnew))

        @pl.when(layer == 1)
        def _():
            pltpu.make_async_copy(io_s.at[_rows(b, RB2), :], out_hbm.at[_rows(b, RB2), :], out_sem.at[b]).start()
        return layer

    def layer_body(layer, carry):
        mt_s[0] = jnp.zeros(mt_s.shape[1:], F32)
        z_s[0] = jnp.zeros(z_s.shape[1:], F32)
        with jax.named_scope('att'):
            lax.fori_loop(0, NU // 2 + 1, att_body, layer)

        @pl.when(layer == 0)
        def _():
            for c in b_copies:
                c.wait()
        with jax.named_scope('out'):
            lax.fori_loop(0, S_ // RB1, out_body, 0)
        with jax.named_scope('mix'):
            lax.fori_loop(0, S_ // RB2, mix_body, layer)
        return carry

    lax.fori_loop(0, 2, layer_body, 0)

    for b in range(S_ // RB2):
        pltpu.make_async_copy(io_s.at[pl.ds(b * RB2, RB2), :], out_hbm.at[pl.ds(b * RB2, RB2), :],
                              out_sem.at[b]).wait()


@jax.jit
def pallas_interleave_layers__memory_aug_infini_attn__mixer_s_mlp__prompt_kernel(
    A_x: jax.Array,
    A_wq: jax.Array,
    A_wk: jax.Array,
    A_wv: jax.Array,
    A_wo: jax.Array,
    A_beta: jax.Array,
    B_x: jax.Array,
    B_w1: jax.Array,
    B_w2: jax.Array,
    B_w3: jax.Array,
    B_w4: jax.Array,
):
    del B_x
    B, S, D = A_x.shape
    assert (B, S, D) == (1, S_, D_) and A_beta.shape == (H_,) and B_w3.shape == (D_, F_)
    hbm = pl.BlockSpec(memory_space=pl.ANY)
    vmem = pl.BlockSpec(memory_space=pltpu.VMEM)
    scratch = [
        pltpu.VMEM((S_, D_), BF16),
        pltpu.VMEM((NG, D_, 128), BF16),
        pltpu.VMEM((NG, D_, 128), BF16),
        pltpu.VMEM((NG, D_, 128), BF16),
        pltpu.VMEM((D_, D_), BF16),
        pltpu.VMEM((D_, D_), BF16),
        pltpu.VMEM((D_, D_), BF16),
        pltpu.VMEM((D_, F_), BF16),
        pltpu.VMEM((F_, D_), BF16),
        pltpu.VMEM((S_, D_), F32),
        pltpu.VMEM((S_, D_), F32),
        pltpu.VMEM((S_ // 2, D_), U32),
        pltpu.VMEM((S_ // 2 + 16, D_), U32),
        pltpu.VMEM((L_ // 2, 256), U32),
        pltpu.VMEM((L_ // 2, 256), U32),
        pltpu.VMEM((L_ // 2, 256), U32),
        pltpu.VMEM((L_ // 2, 256), U32),
        pltpu.VMEM((L_ // 2, 256), U32),
        pltpu.VMEM((L_ // 2, 256), U32),
        pltpu.VMEM((64, L_), U32),
        pltpu.VMEM((64, L_), U32),
        pltpu.VMEM((64, L_), U32),
        pltpu.VMEM((NG, S_ // 2, 128), U32),
        pltpu.VMEM((max(RB1, RB2) // 2, D_), U32),
        pltpu.VMEM((RB2 // 2, D_), U32),
        pltpu.VMEM((RB2, D_), F32),
        pltpu.VMEM((2, NG, 128, 128), F32),
        pltpu.VMEM((2, NG, 8, 128), F32),
        pltpu.VMEM((3, 8, 128), F32),
        pltpu.VMEM((3, 3, 8, 128), F32),
        pltpu.VMEM((H_, 8, 128), F32),
        pltpu.VMEM((RB2 // 4, F_), U32),
        pltpu.SMEM((2,), jnp.int32),
        pltpu.SemaphoreType.DMA((S_ // XB,)),
        pltpu.SemaphoreType.DMA((3, NG)),
        pltpu.SemaphoreType.DMA((5,)),
        pltpu.SemaphoreType.DMA((S_ // RB2,)),
    ]
    out = pl.pallas_call(
        _kernel,
        in_specs=[hbm, hbm, hbm, hbm, hbm, vmem, hbm, hbm, hbm, hbm],
        out_specs=hbm,
        out_shape=jax.ShapeDtypeStruct((S_, D_), BF16),
        scratch_shapes=scratch,
        compiler_params=pltpu.CompilerParams(vmem_limit_bytes=100 * 1024 * 1024),
        name="infini_mixer",
    )(A_x.reshape(S_, D_), A_wq, A_wk, A_wv, A_wo, A_beta.reshape(1, H_), B_w1, B_w2, B_w3, B_w4)
    return out.reshape(1, S_, D_)
```

```python
import numpy as np
import jax
import jax.numpy as jnp
from jax import lax
import jax.experimental.pallas as pl
import jax.experimental.pallas.tpu as pltpu

F32 = jnp.float32
BF16 = jnp.bfloat16
U32 = jnp.uint32

S_, D_, H_, F_ = 2048, 1024, 32, 3584
DH = D_ // H_
NSEG = 4
L_ = S_ // NSEG
NG = D_ // 128
NU = NSEG * NG
EPS = 1e-05
GELU_C0 = float(np.sqrt(2.0 / np.pi))
GELU_C1 = float(0.044715 * np.sqrt(2.0 / np.pi))
QSCALE = float(DH ** -0.5 * np.log2(np.e))
NT = (((1,), (1,)), ((), ()))
ORDER = 3
ORD0='qkv'
ORD1='vqk'
LNC = 16
XB = 256
RB1 = 256
RB2 = 256
LOGIT_BOUND = 60.0
V_BOUND = float(2.0 ** 40)


def _pack(x):
    return pltpu.bitcast(x.astype(BF16), U32)


def _unpack(x):
    return pltpu.bitcast(x, BF16)


def _ln(x):
    m = jnp.sum(x, axis=1, keepdims=True) * (1.0 / D_)
    d = x - m
    v = jnp.sum(d * d, axis=1, keepdims=True) * (1.0 / D_)
    return d * lax.rsqrt(v + EPS)


def _gelu(x):
    t = jnp.tanh(x * (GELU_C0 + GELU_C1 * (x * x)))
    h = 0.5 * x
    return h + h * t


def _phi(t):
    return jnp.where(t > 0, t + 1.0, jnp.exp(t))


def _dot(a, b):
    return jnp.dot(a, b, preferred_element_type=F32)


def _dot_nt(a, b):
    return lax.dot_general(a, b, NT, preferred_element_type=F32)


def _rows(idx, n):
    return pl.ds(pl.multiple_of(idx * n, n), n)


def _kernel(x_hbm, wq_hbm, wk_hbm, wv_hbm, wo_hbm, beta_ref, w1_hbm, w2_hbm, w3_hbm, w4_hbm,
            out_hbm,
            io_s, wq_s, wk_s, wv_s, wo_s, w1_s, w2_s, w3_s, w4_s,
            x_s, xb_s, xn_s, hp_s, qp0_s, qp1_s, qp2_s, kp0_s, kp1_s, kp2_s, vt0_s, vt1_s, vt2_s, o_s, y_s, z2_s, acc_s,
            mt_s, z_s, zk_s, mx_s, g_s, gl_s, flag_s, x_sem, a_sem, b_sem, out_sem):
    def x_copy(b):
        return pltpu.make_async_copy(x_hbm.at[pl.ds(b * XB, XB), :], io_s.at[pl.ds(b * XB, XB), :], x_sem.at[b])

    def a_copies(g):
        cols = pl.ds(pl.multiple_of(g * 128, 128), 128)
        return [pltpu.make_async_copy(w.at[:, cols], ws.at[g], a_sem.at[j, g])
                for j, (w, ws) in enumerate(((wq_hbm, wq_s), (wk_hbm, wk_s), (wv_hbm, wv_s)))]

    b_copies = [pltpu.make_async_copy(a, b, b_sem.at[i]) for i, (a, b) in
                enumerate(((wo_hbm, wo_s), (w1_hbm, w1_s), (w2_hbm, w2_s), (w3_hbm, w3_s), (w4_hbm, w4_s)))]

    for b in range(S_ // XB):
        x_copy(b).start()
    for g in range(2):
        for c in a_copies(g):
            c.start()

    lane = lax.broadcasted_iota(jnp.int32, (8, 128), 1)
    head_mask = [jnp.where((lane >> 5) == h, jnp.uint32(0xFFFFFFFF), jnp.uint32(0)) for h in range(4)]
    rio = lax.broadcasted_iota(jnp.int32, (128, 128), 0)
    cio = lax.broadcasted_iota(jnp.int32, (128, 128), 1)

    bvec = jax.nn.sigmoid(beta_ref[...].astype(F32))
    hio = lax.broadcasted_iota(jnp.int32, (8, H_), 1)
    for h in range(H_):
        gh = jnp.sum(jnp.where(hio == h, bvec, 0.0), axis=1, keepdims=True)
        g_s[h] = jnp.broadcast_to(gh, (8, 128))

    hp_s[0:8, :] = jnp.zeros((8, D_), U32)
    hp_s[8 + S_ // 2:16 + S_ // 2, :] = jnp.zeros((8, D_), U32)

    def prologue(b, c):
        pltpu.make_async_copy(x_hbm.at[_rows(b, XB), :], io_s.at[_rows(b, XB), :], x_sem.at[b]).wait()
        r = _rows(b, XB)
        x = io_s[r, :].astype(F32)
        x_s[r, :] = x
        xn_s[_rows(b, XB // 2), :] = _pack(_ln(x))
        return c
    with jax.named_scope('pro'):
        lax.fori_loop(0, S_ // XB, prologue, 0)

    for g in range(2, NG):
        for c in a_copies(g):
            c.start()
    for c in b_copies[0:2]:
        c.start()

    qp_b, kp_b, vt_b = (qp0_s, qp1_s, qp2_s), (kp0_s, kp1_s, kp2_s), (vt0_s, vt1_s, vt2_s)

    def proj_steps(u, par, order):
        s, g = u >> 3, u & 7
        tok2 = _rows(s, L_ // 2)

        def proj(w_ref):
            return _dot(_unpack(xn_s[tok2, :]), w_ref[g])

        def absmax(a):
            return jnp.max(jnp.abs(a).reshape(L_ // 8, 8, 128), axis=0)

        def step_q():
            q = proj(wq_s)
            qs = q * QSCALE
            qp_b[par][...] = _pack(jnp.concatenate([qs, _phi(q)], axis=1))
            mx_s[par, 0] = absmax(qs)

        def step_k():
            k = proj(wk_s)
            pk = _phi(k)
            kp_b[par][...] = _pack(jnp.concatenate([k, pk], axis=1))
            zk_s[par] = jnp.broadcast_to(jnp.sum(pk, axis=0, keepdims=True), (8, 128))
            mx_s[par, 1] = absmax(k)

        def step_v():
            v = proj(wv_s)
            vt_b[par][...] = pltpu.bitcast(v.astype(BF16).T, U32)
            mx_s[par, 2] = absmax(v)
        return [dict(q=step_q, k=step_k, v=step_v)[c] for c in order]

    def unit_is_safe(par):
        bound = (DH * 1.02) * jnp.max(mx_s[par, 0]) * jnp.max(mx_s[par, 1])
        return jnp.logical_and(bound <= LOGIT_BOUND, jnp.max(mx_s[par, 2]) <= V_BOUND)

    def mem_lhs(s, g):
        mt = jnp.where((rio >> 5) == (cio >> 5), mt_s[s & 1, g], 0.0)
        zr = jnp.where(rio[0:16] == (cio[0:16] >> 5), jnp.broadcast_to(z_s[s & 1, g, 0:1], (16, 128)), 0.0)
        return jnp.concatenate([mt, zr], axis=0).astype(BF16)

    def mem_update(s, g, par):
        mt_s[1 - (s & 1), g] = mt_s[s & 1, g] + _dot(_unpack(vt_b[par][...]), _unpack(kp_b[par][:, 128:256]))
        z_s[1 - (s & 1), g] = z_s[s & 1, g] + zk_s[par]

    def att_unit(u, par, fillers):
        s, g = u >> 3, u & 7
        fillers = list(fillers)
        safe = unit_is_safe(par)

        def fill():
            if fillers:
                fillers.pop(0)()

        def qk(i):
            nk = 128 * (i + 1)
            kk = _unpack(kp_b[par][0:nk // 2, 0:128])
            qu = qp_b[par][i * 64:(i + 1) * 64, 0:128]
            lo, hi = qu[0:32], qu[32:64]
            left = cio[0:1] < 64
            res = []
            for ha in (0, 2):
                ma = jnp.concatenate([head_mask[ha]] * 4, axis=0)
                mb = jnp.concatenate([head_mask[ha + 1]] * 4, axis=0)
                t0 = _dot_nt(kk[0:nk - 64], _unpack(jnp.concatenate([lo & ma, lo & mb], axis=0)))
                t1 = _dot_nt(kk, _unpack(jnp.concatenate([hi & mb, hi & ma], axis=0)))
                tri = rio[0:64] <= (cio[0:64] & 63)
                d0 = jnp.exp2(jnp.where(tri, t0[nk - 128:], -1e30))
                d1 = jnp.exp2(jnp.where(tri, t1[nk - 64:], -1e30))
                e1 = jnp.exp2(t1[:nk - 64])
                e0 = jnp.concatenate([jnp.exp2(t0[:nk - 128]), d0], axis=0) if i > 0 else d0
                pa = jnp.concatenate([jnp.where(left, e0, e1), jnp.where(left, 0.0, d1)], axis=0)
                pb = jnp.concatenate([jnp.where(left, e1, e0), jnp.where(left, d1, 0.0)], axis=0)
                l0 = jnp.sum(e0, axis=0, keepdims=True)
                l1 = jnp.sum(e1, axis=0, keepdims=True) + jnp.sum(d1, axis=0, keepdims=True)
                res.append((pa.astype(BF16), jnp.where(left, l0, l1)))
                res.append((pb.astype(BF16), jnp.where(left, l1, l0)))
            return res

        def pv(i, res):
            nk = 128 * (i + 1)
            outs = []
            for h in range(4):
                p, l = res[h]
                vt = _unpack(vt_b[par][h * 16:(h + 1) * 16, 0:nk])
                o = _dot(vt, p) * (1.0 / l)
                outs.append(pltpu.roll(o, 64, 1) if h & 1 else o)
            return outs

        def finish(i, adot):
            nd = _dot_nt(mem_lhs(s, g), _unpack(qp_b[par][i * 64:(i + 1) * 64, 128:256]))
            inv = 1.0 / (nd[128:136] + 1e-06)
            outs = []
            for h in range(4):
                amem = nd[h * 32:(h + 1) * 32] * jnp.broadcast_to(inv[h:h + 1], (32, 128))
                gh = jnp.concatenate([g_s[g * 4 + h]] * 4, axis=0)
                outs.append(gh * amem + (1.0 - gh) * adot[h])
            ot = jnp.concatenate(outs, axis=0)
            o_s[g, pl.ds(pl.multiple_of(s * (L_ // 2) + i * 64, 64), 64), :] = pltpu.bitcast(
                ot.astype(BF16).T, U32)

        if ORDER == 0:
            fill()
            s3 = qk(3)
            s2 = qk(2)
            finish(3, pv(3, s3))
            fill()
            s1 = qk(1)
            finish(2, pv(2, s2))
            s0 = qk(0)
            finish(1, pv(1, s1))
            finish(0, pv(0, s0))
            fill()
        elif ORDER == 1:
            fill()
            s3 = qk(3)
            s0 = qk(0)
            finish(3, pv(3, s3))
            finish(0, pv(0, s0))
            fill()
            s2 = qk(2)
            s1 = qk(1)
            finish(2, pv(2, s2))
            finish(1, pv(1, s1))
            fill()
        elif ORDER == 3:
            s3 = qk(3)
            s0 = qk(0)
            fill()
            finish(3, pv(3, s3))
            finish(0, pv(0, s0))
            s2 = qk(2)
            s1 = qk(1)
            fill()
            finish(2, pv(2, s2))
            finish(1, pv(1, s1))
            fill()
        elif ORDER == 4:
            s3 = qk(3)
            fill()
            finish(3, pv(3, s3))
            s2 = qk(2)
            fill()
            finish(2, pv(2, s2))
            s1 = qk(1)
            s0 = qk(0)
            fill()
            finish(1, pv(1, s1))
            finish(0, pv(0, s0))
        elif ORDER == 2:
            fill()
            s3 = qk(3)
            fill()
            s2 = qk(2)
            finish(3, pv(3, s3))
            s1 = qk(1)
            finish(2, pv(2, s2))
            s0 = qk(0)
            finish(1, pv(1, s1))
            finish(0, pv(0, s0))
            fill()
        mem_update(s, g, par)
        flag_s[par] = safe.astype(jnp.int32)

    def att_unit_exact(u, par):
        s, g = u >> 3, u & 7
        kk = _unpack(kp_b[par][:, 0:128])
        lhs = mem_lhs(s, g)
        key = lax.broadcasted_iota(jnp.int32, (L_, 128), 0)
        qry = lax.broadcasted_iota(jnp.int32, (L_, 128), 1)

        def tile(i, c):
            rows = pl.ds(pl.multiple_of(i * 64, 64), 64)
            qu = qp_b[par][rows, 0:128]
            nd = _dot_nt(lhs, _unpack(qp_b[par][rows, 128:256]))
            inv = 1.0 / (nd[128:136] + 1e-06)
            outs = []
            for h in range(4):
                qm = _unpack(qu & jnp.concatenate([head_mask[h]] * 8, axis=0))
                st = jnp.where(key <= qry + i * 128, _dot_nt(kk, qm), -1e30)
                p = jnp.exp2(st - jnp.max(st, axis=0, keepdims=True))
                l = jnp.sum(p, axis=0, keepdims=True)
                adot = _dot(_unpack(vt_b[par][h * 16:(h + 1) * 16, :]), p.astype(BF16)) * (1.0 / l)
                amem = nd[h * 32:(h + 1) * 32] * jnp.broadcast_to(inv[h:h + 1], (32, 128))
                gh = jnp.concatenate([g_s[g * 4 + h]] * 4, axis=0)
                outs.append(gh * amem + (1.0 - gh) * adot)
            ot = jnp.concatenate(outs, axis=0)
            o_s[g, pl.ds(pl.multiple_of(s * (L_ // 2) + i * 64, 64), 64), :] = pltpu.bitcast(
                ot.astype(BF16).T, U32)
            return c
        lax.fori_loop(0, 4, tile, 0)

    def att_body(t, layer):
        NT_ = NU // 2
        ua = jnp.maximum(2 * t - 1, 1)
        ub = jnp.minimum(2 * t, NU - 2)

        @pl.when(jnp.logical_and(layer == 0, t < NG // 2))
        def _():
            for c in a_copies(2 * t) + a_copies(2 * t + 1):
                c.wait()

        @pl.when(jnp.logical_and(layer == 0, t == 2))
        def _():
            for c in b_copies[2:]:
                c.start()

        @pl.when(t == 0)
        def _():
            for st in proj_steps(ub, 0, 'qkv'):
                st()
            flag_s[1] = 1
            att_unit(ub, 0, proj_steps(ub + 1, 1, ORD1))

        @pl.when(jnp.logical_and(t > 0, t < NT_))
        def _():
            att_unit(ua, 1, proj_steps(ub, 0, ORD0))
            att_unit(ub, 0, proj_steps(ub + 1, 1, ORD1))

        @pl.when(t == NT_)
        def _():
            att_unit(ua, 1, [])
            flag_s[0] = 1

        def redo(j, c):
            @pl.when(flag_s[j] == 0)
            def _():
                u = jnp.where(j == 0, ub, ua)
                for st in proj_steps(u, 2, 'qkv'):
                    st()
                att_unit_exact(u, 2)
            return c
        lax.fori_loop(0, 2, redo, 0)
        return layer

    def out_body(b, c):
        hb = RB1 // 2
        for hf in range(2):
            r = pl.ds(pl.multiple_of(b * RB1 + hf * hb, hb), hb)
            r2 = pl.ds(pl.multiple_of(b * (RB1 // 2) + hf * (hb // 2), hb // 2), hb // 2)
            o = jnp.concatenate([o_s[g, r2, :] for g in range(NG)], axis=1)
            x_s[r, :] = x_s[r, :] + _dot(_unpack(o), wo_s[...])
            for j in range(1):
                LNC = hb
                rj = pl.ds(pl.multiple_of(b * RB1 + hf * hb + j * LNC, LNC), LNC)
                xb = _ln(x_s[rj, :])
                xb_s[rj, :] = xb
                y_s[pl.ds(hf * (hb // 2) + j * (LNC // 2), LNC // 2), :] = _pack(_ln(xb))
        for hf in range(2):
            h = _gelu(_dot(_unpack(y_s[hf * (hb // 2):(hf + 1) * (hb // 2), :]), w1_s[...]))
            hp_s[pl.ds(pl.multiple_of(8 + b * (RB1 // 2) + hf * (hb // 2), 8), hb // 2), :] = _pack(h)
        return c

    def next_ln(hblk):
        hb = RB2 // 2
        for j in range(hb // LNC):
            rj = pl.ds(pl.multiple_of(hblk * hb + j * LNC, LNC), LNC)
            xn_s[pl.ds(pl.multiple_of(hblk * (hb // 2) + j * (LNC // 2), LNC // 2), LNC // 2), :] = _pack(_ln(x_s[rj, :]))

    def mix_body(b, layer):
        n2 = RB2 // 2
        base = pl.multiple_of(b * n2, 8)

        def shifted(c):
            w = hp_s[pl.ds(base, n2 + 16), c * 256:(c + 1) * 256]
            cur = w[8:8 + n2]
            if c == 0:
                return (w[7:7 + n2] >> 16) | (cur << 16)
            if c == 1:
                return (cur >> 16) | (w[9:9 + n2] << 16)
            if c == 2:
                return w[7:7 + n2]
            return w[9:9 + n2]

        next_ln(jnp.maximum(2 * b - 1, 0))
        for c in range(4):
            y_s[0:n2, c * 256:(c + 1) * 256] = shifted(c)
        hb = RB2 // 2
        h2r = hb // 2
        for hf in range(2):
            r = pl.ds(pl.multiple_of(b * RB2 + hf * hb, hb), hb)
            x1 = xb_s[r, :] + _dot(_unpack(y_s[hf * h2r:(hf + 1) * h2r, :]), w2_s[...])
            acc_s[hf * hb:(hf + 1) * hb, :] = x1
            for j in range(hb // LNC):
                z2_s[pl.ds(hf * h2r + j * (LNC // 2), LNC // 2), :] = _pack(_ln(acc_s[pl.ds(hf * hb + j * LNC, LNC), :]))
        for hf in range(2):
            r = pl.ds(pl.multiple_of(b * RB2 + hf * hb, hb), hb)
            z = _unpack(z2_s[hf * h2r:(hf + 1) * h2r, :])
            for ch in range(F_ // 512):
                gl_s[:, ch * 512:(ch + 1) * 512] = _pack(_gelu(_dot(z, w3_s[:, ch * 512:(ch + 1) * 512])))
            h2 = _dot(_unpack(gl_s[...]), w4_s[...])
            xnew = x_s[r, :] + (acc_s[hf * hb:(hf + 1) * hb, :] + h2)
            x_s[r, :] = xnew
            io_s[r, :] = xnew.astype(BF16)
            if hf == 0:
                next_ln(2 * b)

        @pl.when(layer == 1)
        def _():
            pltpu.make_async_copy(io_s.at[_rows(b, RB2), :], out_hbm.at[_rows(b, RB2), :], out_sem.at[b]).start()
        return layer

    def layer_body(layer, carry):
        mt_s[0] = jnp.zeros(mt_s.shape[1:], F32)
        z_s[0] = jnp.zeros(z_s.shape[1:], F32)
        with jax.named_scope('att'):
            lax.fori_loop(0, NU // 2 + 1, att_body, layer)

        @pl.when(layer == 0)
        def _():
            with jax.named_scope('bw'):
              for c in b_copies:
                c.wait()
        with jax.named_scope('out'):
            lax.fori_loop(0, S_ // RB1, out_body, 0)
        with jax.named_scope('mix'):
            lax.fori_loop(0, S_ // RB2, mix_body, layer)

        @pl.when(layer == 0)
        def _():
            next_ln(2 * (S_ // RB2) - 1)
        return carry

    lax.fori_loop(0, 2, layer_body, 0)

    with jax.named_scope('fin'):
      for b in range(S_ // RB2):
        pltpu.make_async_copy(io_s.at[pl.ds(b * RB2, RB2), :], out_hbm.at[pl.ds(b * RB2, RB2), :],
                              out_sem.at[b]).wait()


@jax.jit
def pallas_interleave_layers__memory_aug_infini_attn__mixer_s_mlp__prompt_kernel(
    A_x: jax.Array,
    A_wq: jax.Array,
    A_wk: jax.Array,
    A_wv: jax.Array,
    A_wo: jax.Array,
    A_beta: jax.Array,
    B_x: jax.Array,
    B_w1: jax.Array,
    B_w2: jax.Array,
    B_w3: jax.Array,
    B_w4: jax.Array,
):
    del B_x
    B, S, D = A_x.shape
    assert (B, S, D) == (1, S_, D_) and A_beta.shape == (H_,) and B_w3.shape == (D_, F_)
    hbm = pl.BlockSpec(memory_space=pl.ANY)
    vmem = pl.BlockSpec(memory_space=pltpu.VMEM)
    scratch = [
        pltpu.VMEM((S_, D_), BF16),
        pltpu.VMEM((NG, D_, 128), BF16),
        pltpu.VMEM((NG, D_, 128), BF16),
        pltpu.VMEM((NG, D_, 128), BF16),
        pltpu.VMEM((D_, D_), BF16),
        pltpu.VMEM((D_, D_), BF16),
        pltpu.VMEM((D_, D_), BF16),
        pltpu.VMEM((D_, F_), BF16),
        pltpu.VMEM((F_, D_), BF16),
        pltpu.VMEM((S_, D_), F32),
        pltpu.VMEM((S_, D_), F32),
        pltpu.VMEM((S_ // 2, D_), U32),
        pltpu.VMEM((S_ // 2 + 16, D_), U32),
        pltpu.VMEM((L_ // 2, 256), U32),
        pltpu.VMEM((L_ // 2, 256), U32),
        pltpu.VMEM((L_ // 2, 256), U32),
        pltpu.VMEM((L_ // 2, 256), U32),
        pltpu.VMEM((L_ // 2, 256), U32),
        pltpu.VMEM((L_ // 2, 256), U32),
        pltpu.VMEM((64, L_), U32),
        pltpu.VMEM((64, L_), U32),
        pltpu.VMEM((64, L_), U32),
        pltpu.VMEM((NG, S_ // 2, 128), U32),
        pltpu.VMEM((max(RB1, RB2) // 2, D_), U32),
        pltpu.VMEM((RB2 // 2, D_), U32),
        pltpu.VMEM((RB2, D_), F32),
        pltpu.VMEM((2, NG, 128, 128), F32),
        pltpu.VMEM((2, NG, 8, 128), F32),
        pltpu.VMEM((3, 8, 128), F32),
        pltpu.VMEM((3, 3, 8, 128), F32),
        pltpu.VMEM((H_, 8, 128), F32),
        pltpu.VMEM((RB2 // 4, F_), U32),
        pltpu.SMEM((2,), jnp.int32),
        pltpu.SemaphoreType.DMA((S_ // XB,)),
        pltpu.SemaphoreType.DMA((3, NG)),
        pltpu.SemaphoreType.DMA((5,)),
        pltpu.SemaphoreType.DMA((S_ // RB2,)),
    ]
    out = pl.pallas_call(
        _kernel,
        in_specs=[hbm, hbm, hbm, hbm, hbm, vmem, hbm, hbm, hbm, hbm],
        out_specs=hbm,
        out_shape=jax.ShapeDtypeStruct((S_, D_), BF16),
        scratch_shapes=scratch,
        compiler_params=pltpu.CompilerParams(vmem_limit_bytes=100 * 1024 * 1024),
        name="infini_mixer",
    )(A_x.reshape(S_, D_), A_wq, A_wk, A_wv, A_wo, A_beta.reshape(1, H_), B_w1, B_w2, B_w3, B_w4)
    return out.reshape(1, S_, D_)
```

```python
import numpy as np
import jax
import jax.numpy as jnp
from jax import lax
import jax.experimental.pallas as pl
import jax.experimental.pallas.tpu as pltpu

F32 = jnp.float32
BF16 = jnp.bfloat16
U32 = jnp.uint32

S_, D_, H_, F_ = 2048, 1024, 32, 3584
DH = D_ // H_
NSEG = 4
L_ = S_ // NSEG
NG = D_ // 128
NU = NSEG * NG
EPS = 1e-05
GELU_C0 = float(np.sqrt(2.0 / np.pi))
GELU_C1 = float(0.044715 * np.sqrt(2.0 / np.pi))
QSCALE = float(DH ** -0.5 * np.log2(np.e))
NT = (((1,), (1,)), ((), ()))
ORD0, ORD1 = 'qkv', 'vqk'
LNC = 16
XB = 256
RB1 = 256
RB2 = 256
LOGIT_BOUND = 60.0
V_BOUND = float(2.0 ** 40)


def _pack(x):
    return pltpu.bitcast(x.astype(BF16), U32)


def _unpack(x):
    return pltpu.bitcast(x, BF16)


def _ln(x):
    m = jnp.sum(x, axis=1, keepdims=True) * (1.0 / D_)
    d = x - m
    v = jnp.sum(d * d, axis=1, keepdims=True) * (1.0 / D_)
    return d * lax.rsqrt(v + EPS)


def _gelu(x):
    t = jnp.tanh(x * (GELU_C0 + GELU_C1 * (x * x)))
    h = 0.5 * x
    return h + h * t


def _phi(t):
    return jnp.where(t > 0, t + 1.0, jnp.exp(t))


def _dot(a, b):
    return jnp.dot(a, b, preferred_element_type=F32)


def _dot_nt(a, b):
    return lax.dot_general(a, b, NT, preferred_element_type=F32)


def _rows(idx, n):
    return pl.ds(pl.multiple_of(idx * n, n), n)


def _kernel(x_hbm, wq_hbm, wk_hbm, wv_hbm, wo_hbm, beta_ref, w1_hbm, w2_hbm, w3_hbm, w4_hbm,
            out_hbm,
            io_s, wq_s, wk_s, wv_s, wo_s, w1_s, w2_s, w3_s, w4_s,
            x_s, xb_s, xn_s, hp_s, qp0_s, qp1_s, qp2_s, kp0_s, kp1_s, kp2_s, vt0_s, vt1_s, vt2_s, o_s, y_s, z2_s, acc_s,
            mt_s, z_s, zk_s, mx_s, g_s, gl_s, flag_s, x_sem, a_sem, b_sem, out_sem):
    def x_copy(b):
        return pltpu.make_async_copy(x_hbm.at[pl.ds(b * XB, XB), :], io_s.at[pl.ds(b * XB, XB), :], x_sem.at[b])

    def a_copies(g):
        cols = pl.ds(pl.multiple_of(g * 128, 128), 128)
        return [pltpu.make_async_copy(w.at[:, cols], ws.at[g], a_sem.at[j, g])
                for j, (w, ws) in enumerate(((wq_hbm, wq_s), (wk_hbm, wk_s), (wv_hbm, wv_s)))]

    b_copies = [pltpu.make_async_copy(a, b, b_sem.at[i]) for i, (a, b) in
                enumerate(((wo_hbm, wo_s), (w1_hbm, w1_s), (w2_hbm, w2_s), (w3_hbm, w3_s), (w4_hbm, w4_s)))]

    for b in range(S_ // XB):
        x_copy(b).start()
    for g in range(2):
        for c in a_copies(g):
            c.start()

    lane = lax.broadcasted_iota(jnp.int32, (8, 128), 1)
    head_mask = [jnp.where((lane >> 5) == h, jnp.uint32(0xFFFFFFFF), jnp.uint32(0)) for h in range(4)]
    rio = lax.broadcasted_iota(jnp.int32, (128, 128), 0)
    cio = lax.broadcasted_iota(jnp.int32, (128, 128), 1)

    bvec = jax.nn.sigmoid(beta_ref[...].astype(F32))
    hio = lax.broadcasted_iota(jnp.int32, (8, H_), 1)
    for h in range(H_):
        gh = jnp.sum(jnp.where(hio == h, bvec, 0.0), axis=1, keepdims=True)
        g_s[h] = jnp.broadcast_to(gh, (8, 128))

    hp_s[0:8, :] = jnp.zeros((8, D_), U32)
    hp_s[8 + S_ // 2:16 + S_ // 2, :] = jnp.zeros((8, D_), U32)

    def prologue(b, c):
        pltpu.make_async_copy(x_hbm.at[_rows(b, XB), :], io_s.at[_rows(b, XB), :], x_sem.at[b]).wait()
        r = _rows(b, XB)
        x = io_s[r, :].astype(F32)
        x_s[r, :] = x
        xn_s[_rows(b, XB // 2), :] = _pack(_ln(x))
        return c
    lax.fori_loop(0, S_ // XB, prologue, 0)

    for g in range(2, NG):
        for c in a_copies(g):
            c.start()
    for c in b_copies[0:2]:
        c.start()

    qp_b, kp_b, vt_b = (qp0_s, qp1_s, qp2_s), (kp0_s, kp1_s, kp2_s), (vt0_s, vt1_s, vt2_s)

    def proj_steps(u, par, order):
        s, g = u >> 3, u & 7
        tok2 = _rows(s, L_ // 2)

        def proj(w_ref):
            return _dot(_unpack(xn_s[tok2, :]), w_ref[g])

        def absmax(a):
            return jnp.max(jnp.abs(a).reshape(L_ // 8, 8, 128), axis=0)

        def step_q():
            q = proj(wq_s)
            qs = q * QSCALE
            qp_b[par][...] = _pack(jnp.concatenate([qs, _phi(q)], axis=1))
            mx_s[par, 0] = absmax(qs)

        def step_k():
            k = proj(wk_s)
            pk = _phi(k)
            kp_b[par][...] = _pack(jnp.concatenate([k, pk], axis=1))
            zk_s[par] = jnp.broadcast_to(jnp.sum(pk, axis=0, keepdims=True), (8, 128))
            mx_s[par, 1] = absmax(k)

        def step_v():
            v = proj(wv_s)
            vt_b[par][...] = pltpu.bitcast(v.astype(BF16).T, U32)
            mx_s[par, 2] = absmax(v)
        return [dict(q=step_q, k=step_k, v=step_v)[c] for c in order]

    def unit_is_safe(par):
        bound = (DH * 1.02) * jnp.max(mx_s[par, 0]) * jnp.max(mx_s[par, 1])
        return jnp.logical_and(bound <= LOGIT_BOUND, jnp.max(mx_s[par, 2]) <= V_BOUND)

    def mem_lhs(s, g):
        mt = jnp.where((rio >> 5) == (cio >> 5), mt_s[s & 1, g], 0.0)
        zr = jnp.where(rio[0:16] == (cio[0:16] >> 5), jnp.broadcast_to(z_s[s & 1, g, 0:1], (16, 128)), 0.0)
        return jnp.concatenate([mt, zr], axis=0).astype(BF16)

    def mem_update(s, g, par):
        mt_s[1 - (s & 1), g] = mt_s[s & 1, g] + _dot(_unpack(vt_b[par][...]), _unpack(kp_b[par][:, 128:256]))
        z_s[1 - (s & 1), g] = z_s[s & 1, g] + zk_s[par]

    def att_unit(u, par, fillers):
        s, g = u >> 3, u & 7
        fillers = list(fillers)
        safe = unit_is_safe(par)

        def fill():
            if fillers:
                fillers.pop(0)()

        def qk(i):
            nk = 128 * (i + 1)
            kk = _unpack(kp_b[par][0:nk // 2, 0:128])
            qu = qp_b[par][i * 64:(i + 1) * 64, 0:128]
            lo, hi = qu[0:32], qu[32:64]
            left = cio[0:1] < 64
            res = []
            for ha in (0, 2):
                ma = jnp.concatenate([head_mask[ha]] * 4, axis=0)
                mb = jnp.concatenate([head_mask[ha + 1]] * 4, axis=0)
                t0 = _dot_nt(kk[0:nk - 64], _unpack(jnp.concatenate([lo & ma, lo & mb], axis=0)))
                t1 = _dot_nt(kk, _unpack(jnp.concatenate([hi & mb, hi & ma], axis=0)))
                tri = rio[0:64] <= (cio[0:64] & 63)
                d0 = jnp.exp2(jnp.where(tri, t0[nk - 128:], -1e30))
                d1 = jnp.exp2(jnp.where(tri, t1[nk - 64:], -1e30))
                e1 = jnp.exp2(t1[:nk - 64])
                e0 = jnp.concatenate([jnp.exp2(t0[:nk - 128]), d0], axis=0) if i > 0 else d0
                pa = jnp.concatenate([jnp.where(left, e0, e1), jnp.where(left, 0.0, d1)], axis=0)
                pb = jnp.concatenate([jnp.where(left, e1, e0), jnp.where(left, d1, 0.0)], axis=0)
                l0 = jnp.sum(e0, axis=0, keepdims=True)
                l1 = jnp.sum(e1, axis=0, keepdims=True) + jnp.sum(d1, axis=0, keepdims=True)
                res.append((pa.astype(BF16), jnp.where(left, l0, l1)))
                res.append((pb.astype(BF16), jnp.where(left, l1, l0)))
            return res

        def pv(i, res):
            nk = 128 * (i + 1)
            outs = []
            for h in range(4):
                p, l = res[h]
                vt = _unpack(vt_b[par][h * 16:(h + 1) * 16, 0:nk])
                o = _dot(vt, p) * (1.0 / l)
                outs.append(pltpu.roll(o, 64, 1) if h & 1 else o)
            return outs

        def finish(i, adot):
            nd = _dot_nt(mem_lhs(s, g), _unpack(qp_b[par][i * 64:(i + 1) * 64, 128:256]))
            inv = 1.0 / (nd[128:136] + 1e-06)
            outs = []
            for h in range(4):
                amem = nd[h * 32:(h + 1) * 32] * jnp.broadcast_to(inv[h:h + 1], (32, 128))
                gh = jnp.concatenate([g_s[g * 4 + h]] * 4, axis=0)
                outs.append(gh * amem + (1.0 - gh) * adot[h])
            ot = jnp.concatenate(outs, axis=0)
            o_s[g, pl.ds(pl.multiple_of(s * (L_ // 2) + i * 64, 64), 64), :] = pltpu.bitcast(
                ot.astype(BF16).T, U32)

        s3 = qk(3)
        s0 = qk(0)
        fill()
        finish(3, pv(3, s3))
        finish(0, pv(0, s0))
        s2 = qk(2)
        s1 = qk(1)
        fill()
        finish(2, pv(2, s2))
        finish(1, pv(1, s1))
        fill()
        mem_update(s, g, par)
        flag_s[par] = safe.astype(jnp.int32)

    def att_unit_exact(u, par):
        s, g = u >> 3, u & 7
        kk = _unpack(kp_b[par][:, 0:128])
        lhs = mem_lhs(s, g)
        key = lax.broadcasted_iota(jnp.int32, (L_, 128), 0)
        qry = lax.broadcasted_iota(jnp.int32, (L_, 128), 1)

        def tile(i, c):
            rows = pl.ds(pl.multiple_of(i * 64, 64), 64)
            qu = qp_b[par][rows, 0:128]
            nd = _dot_nt(lhs, _unpack(qp_b[par][rows, 128:256]))
            inv = 1.0 / (nd[128:136] + 1e-06)
            outs = []
            for h in range(4):
                qm = _unpack(qu & jnp.concatenate([head_mask[h]] * 8, axis=0))
                st = jnp.where(key <= qry + i * 128, _dot_nt(kk, qm), -1e30)
                p = jnp.exp2(st - jnp.max(st, axis=0, keepdims=True))
                l = jnp.sum(p, axis=0, keepdims=True)
                adot = _dot(_unpack(vt_b[par][h * 16:(h + 1) * 16, :]), p.astype(BF16)) * (1.0 / l)
                amem = nd[h * 32:(h + 1) * 32] * jnp.broadcast_to(inv[h:h + 1], (32, 128))
                gh = jnp.concatenate([g_s[g * 4 + h]] * 4, axis=0)
                outs.append(gh * amem + (1.0 - gh) * adot)
            ot = jnp.concatenate(outs, axis=0)
            o_s[g, pl.ds(pl.multiple_of(s * (L_ // 2) + i * 64, 64), 64), :] = pltpu.bitcast(
                ot.astype(BF16).T, U32)
            return c
        lax.fori_loop(0, 4, tile, 0)

    def att_body(t, layer):
        NT_ = NU // 2
        ua = jnp.maximum(2 * t - 1, 1)
        ub = jnp.minimum(2 * t, NU - 2)

        @pl.when(jnp.logical_and(layer == 0, t < NG // 2))
        def _():
            for c in a_copies(2 * t) + a_copies(2 * t + 1):
                c.wait()

        @pl.when(jnp.logical_and(layer == 0, t == 2))
        def _():
            for c in b_copies[2:]:
                c.start()

        @pl.when(t == 0)
        def _():
            for st in proj_steps(ub, 0, 'qkv'):
                st()
            flag_s[1] = 1
            att_unit(ub, 0, proj_steps(ub + 1, 1, ORD1))

        @pl.when(jnp.logical_and(t > 0, t < NT_))
        def _():
            att_unit(ua, 1, proj_steps(ub, 0, ORD0))
            att_unit(ub, 0, proj_steps(ub + 1, 1, ORD1))

        @pl.when(t == NT_)
        def _():
            att_unit(ua, 1, [])
            flag_s[0] = 1

        def redo(j, c):
            @pl.when(flag_s[j] == 0)
            def _():
                u = jnp.where(j == 0, ub, ua)
                for st in proj_steps(u, 2, 'qkv'):
                    st()
                att_unit_exact(u, 2)
            return c
        lax.fori_loop(0, 2, redo, 0)
        return layer

    def out_body(b, c):
        hb = RB1 // 2
        for hf in range(2):
            r = pl.ds(pl.multiple_of(b * RB1 + hf * hb, hb), hb)
            r2 = pl.ds(pl.multiple_of(b * (RB1 // 2) + hf * (hb // 2), hb // 2), hb // 2)
            o = jnp.concatenate([o_s[g, r2, :] for g in range(NG)], axis=1)
            x_s[r, :] = x_s[r, :] + _dot(_unpack(o), wo_s[...])
            for j in range(1):
                LNC = hb
                rj = pl.ds(pl.multiple_of(b * RB1 + hf * hb + j * LNC, LNC), LNC)
                xb = _ln(x_s[rj, :])
                xb_s[rj, :] = xb
                y_s[pl.ds(hf * (hb // 2) + j * (LNC // 2), LNC // 2), :] = _pack(_ln(xb))
        for hf in range(2):
            h = _gelu(_dot(_unpack(y_s[hf * (hb // 2):(hf + 1) * (hb // 2), :]), w1_s[...]))
            hp_s[pl.ds(pl.multiple_of(8 + b * (RB1 // 2) + hf * (hb // 2), 8), hb // 2), :] = _pack(h)
        return c

    def next_ln(hblk):
        hb = RB2 // 2
        for j in range(hb // LNC):
            rj = pl.ds(pl.multiple_of(hblk * hb + j * LNC, LNC), LNC)
            xn_s[pl.ds(pl.multiple_of(hblk * (hb // 2) + j * (LNC // 2), LNC // 2), LNC // 2), :] = _pack(_ln(x_s[rj, :]))

    def mix_body(b, layer):
        n2 = RB2 // 2
        base = pl.multiple_of(b * n2, 8)

        def shifted(c):
            w = hp_s[pl.ds(base, n2 + 16), c * 256:(c + 1) * 256]
            cur = w[8:8 + n2]
            if c == 0:
                return (w[7:7 + n2] >> 16) | (cur << 16)
            if c == 1:
                return (cur >> 16) | (w[9:9 + n2] << 16)
            if c == 2:
                return w[7:7 + n2]
            return w[9:9 + n2]

        next_ln(jnp.maximum(2 * b - 1, 0))
        for c in range(4):
            y_s[0:n2, c * 256:(c + 1) * 256] = shifted(c)
        hb = RB2 // 2
        h2r = hb // 2
        for hf in range(2):
            r = pl.ds(pl.multiple_of(b * RB2 + hf * hb, hb), hb)
            x1 = xb_s[r, :] + _dot(_unpack(y_s[hf * h2r:(hf + 1) * h2r, :]), w2_s[...])
            acc_s[hf * hb:(hf + 1) * hb, :] = x1
            for j in range(hb // LNC):
                z2_s[pl.ds(hf * h2r + j * (LNC // 2), LNC // 2), :] = _pack(_ln(acc_s[pl.ds(hf * hb + j * LNC, LNC), :]))
        for hf in range(2):
            r = pl.ds(pl.multiple_of(b * RB2 + hf * hb, hb), hb)
            z = _unpack(z2_s[hf * h2r:(hf + 1) * h2r, :])
            for ch in range(F_ // 512):
                gl_s[:, ch * 512:(ch + 1) * 512] = _pack(_gelu(_dot(z, w3_s[:, ch * 512:(ch + 1) * 512])))
            h2 = _dot(_unpack(gl_s[...]), w4_s[...])
            xnew = x_s[r, :] + (acc_s[hf * hb:(hf + 1) * hb, :] + h2)
            x_s[r, :] = xnew
            io_s[r, :] = xnew.astype(BF16)
            if hf == 0:
                next_ln(2 * b)

        @pl.when(layer == 1)
        def _():
            pltpu.make_async_copy(io_s.at[_rows(b, RB2), :], out_hbm.at[_rows(b, RB2), :], out_sem.at[b]).start()
        return layer

    def layer_body(layer, carry):
        mt_s[0] = jnp.zeros(mt_s.shape[1:], F32)
        z_s[0] = jnp.zeros(z_s.shape[1:], F32)
        lax.fori_loop(0, NU // 2 + 1, att_body, layer)

        @pl.when(layer == 0)
        def _():
            for c in b_copies:
              c.wait()
        lax.fori_loop(0, S_ // RB1, out_body, 0)
        lax.fori_loop(0, S_ // RB2, mix_body, layer)

        @pl.when(layer == 0)
        def _():
            next_ln(2 * (S_ // RB2) - 1)
        return carry

    lax.fori_loop(0, 2, layer_body, 0)

    for b in range(S_ // RB2):
      pltpu.make_async_copy(io_s.at[pl.ds(b * RB2, RB2), :], out_hbm.at[pl.ds(b * RB2, RB2), :],
                            out_sem.at[b]).wait()


@jax.jit
def pallas_interleave_layers__memory_aug_infini_attn__mixer_s_mlp__prompt_kernel(
    A_x: jax.Array,
    A_wq: jax.Array,
    A_wk: jax.Array,
    A_wv: jax.Array,
    A_wo: jax.Array,
    A_beta: jax.Array,
    B_x: jax.Array,
    B_w1: jax.Array,
    B_w2: jax.Array,
    B_w3: jax.Array,
    B_w4: jax.Array,
):
    del B_x
    B, S, D = A_x.shape
    assert (B, S, D) == (1, S_, D_) and A_beta.shape == (H_,) and B_w3.shape == (D_, F_)
    hbm = pl.BlockSpec(memory_space=pl.ANY)
    vmem = pl.BlockSpec(memory_space=pltpu.VMEM)
    scratch = [
        pltpu.VMEM((S_, D_), BF16),
        pltpu.VMEM((NG, D_, 128), BF16),
        pltpu.VMEM((NG, D_, 128), BF16),
        pltpu.VMEM((NG, D_, 128), BF16),
        pltpu.VMEM((D_, D_), BF16),
        pltpu.VMEM((D_, D_), BF16),
        pltpu.VMEM((D_, D_), BF16),
        pltpu.VMEM((D_, F_), BF16),
        pltpu.VMEM((F_, D_), BF16),
        pltpu.VMEM((S_, D_), F32),
        pltpu.VMEM((S_, D_), F32),
        pltpu.VMEM((S_ // 2, D_), U32),
        pltpu.VMEM((S_ // 2 + 16, D_), U32),
        pltpu.VMEM((L_ // 2, 256), U32),
        pltpu.VMEM((L_ // 2, 256), U32),
        pltpu.VMEM((L_ // 2, 256), U32),
        pltpu.VMEM((L_ // 2, 256), U32),
        pltpu.VMEM((L_ // 2, 256), U32),
        pltpu.VMEM((L_ // 2, 256), U32),
        pltpu.VMEM((64, L_), U32),
        pltpu.VMEM((64, L_), U32),
        pltpu.VMEM((64, L_), U32),
        pltpu.VMEM((NG, S_ // 2, 128), U32),
        pltpu.VMEM((max(RB1, RB2) // 2, D_), U32),
        pltpu.VMEM((RB2 // 2, D_), U32),
        pltpu.VMEM((RB2, D_), F32),
        pltpu.VMEM((2, NG, 128, 128), F32),
        pltpu.VMEM((2, NG, 8, 128), F32),
        pltpu.VMEM((3, 8, 128), F32),
        pltpu.VMEM((3, 3, 8, 128), F32),
        pltpu.VMEM((H_, 8, 128), F32),
        pltpu.VMEM((RB2 // 4, F_), U32),
        pltpu.SMEM((2,), jnp.int32),
        pltpu.SemaphoreType.DMA((S_ // XB,)),
        pltpu.SemaphoreType.DMA((3, NG)),
        pltpu.SemaphoreType.DMA((5,)),
        pltpu.SemaphoreType.DMA((S_ // RB2,)),
    ]
    out = pl.pallas_call(
        _kernel,
        in_specs=[hbm, hbm, hbm, hbm, hbm, vmem, hbm, hbm, hbm, hbm],
        out_specs=hbm,
        out_shape=jax.ShapeDtypeStruct((S_, D_), BF16),
        scratch_shapes=scratch,
        compiler_params=pltpu.CompilerParams(vmem_limit_bytes=100 * 1024 * 1024),
        name="infini_mixer",
    )(A_x.reshape(S_, D_), A_wq, A_wk, A_wv, A_wo, A_beta.reshape(1, H_), B_w1, B_w2, B_w3, B_w4)
    return out.reshape(1, S_, D_)
```
